```python
import jax
import jax.numpy as jnp

def _softmax(x, axis=-1):
    return jax.nn.softmax(x, axis=axis)
def _gelu(x):
    return jax.nn.gelu(x, approximate=True)
def _silu(x):
    return jax.nn.silu(x)
def _sigmoid(x):
    return jax.nn.sigmoid(x)
def _layernorm(x, axis=-1, eps=1e-5):
    m = jnp.mean(x, axis=axis, keepdims=True)
    v = jnp.var(x, axis=axis, keepdims=True)
    return (x - m) / jnp.sqrt(v + eps)
def _scatter_add(tgt, idx, src, axis=0):
    return tgt.at[idx].add(src)
def _segment_sum(src, seg, n):
    return jax.ops.segment_sum(src, seg, n)
class _Rng:
    def __init__(self, key):
        self._k = key
    def _next(self):
        self._k, sub = jax.random.split(self._k)
        return sub
    def normal(self, shape):
        return jax.random.normal(self._next(), shape, dtype=jnp.bfloat16)
    def randint(self, lo, hi, shape):
        return jax.random.randint(self._next(), shape, lo, hi, dtype=jnp.int32)
    def uniform(self, shape, lo=0.0, hi=1.0):
        return jax.random.uniform(self._next(), shape, jnp.bfloat16, lo, hi)
    def permutation(self, n):
        return jax.random.permutation(self._next(), n)


kernel_name = 'recurrent_scan__compressed_kv_cla__dense_activation_gelu__decode'

def setup_inputs():
    _rng = _Rng(jax.random.key(int.from_bytes(__import__("os").urandom(4), "little")))
    _w = (lambda a: (lambda t: t.astype(jnp.bfloat16) if jnp.issubdtype(t.dtype, jnp.floating) else t)(jnp.asarray(a)))
    def _A_setup():
        B, H, Sq, Sk, D, M = 2, 32, 1, 16384, 128, 512
        Dc = 4 * D
        return {
            "x": _w((lambda *s: _rng.normal(s) * 0.05)(B, Sq, M)),
            "c_kv": _w((lambda *s: _rng.normal(s) * 0.05)(B, Sk, Dc)),
            "w_q": _w((lambda *s: _rng.normal(s) * 0.05)(M, H, D) * (M ** -0.5)),
            "w_uk": _w((lambda *s: _rng.normal(s) * 0.05)(Dc, H, D) * (Dc ** -0.5)),
            "w_uv": _w((lambda *s: _rng.normal(s) * 0.05)(Dc, H, D) * (Dc ** -0.5)),
            "w_o": _w((lambda *s: _rng.normal(s) * 0.05)(H, D, M) * ((H * D) ** -0.5)),
        }
    _A_in = _A_setup()

    def _B_setup():
        B, S, D, F = 2, 1, 512, 1792
        return {
            "x": _w((lambda *s: _rng.normal(s) * 0.05)(B, S, D)),
            "w1": _w((lambda *s: _rng.normal(s) * 0.05)(D, F) * (D ** -0.5)),
            "b1": _w((lambda *s: _rng.normal(s) * 0.05)(F) * 0.01),
            "w2": _w((lambda *s: _rng.normal(s) * 0.05)(F, D) * (F ** -0.5)),
            "b2": _w((lambda *s: _rng.normal(s) * 0.05)(D) * 0.01),
        }
    _B_in = _B_setup()

    return {
        "A_x": _A_in["x"],
        "A_c_kv": _A_in["c_kv"],
        "A_w_q": _A_in["w_q"],
        "A_w_uk": _A_in["w_uk"],
        "A_w_uv": _A_in["w_uv"],
        "A_w_o": _A_in["w_o"],
        "B_x": _B_in["x"],
        "B_w1": _B_in["w1"],
        "B_b1": _B_in["b1"],
        "B_w2": _B_in["w2"],
        "B_b2": _B_in["b2"],
    }

def reference(A_x, A_c_kv, A_w_q, A_w_uk, A_w_uv, A_w_o, B_x, B_w1, B_b1, B_w2, B_b2):
    def _A_ref(x, c_kv, w_q, w_uk, w_uv, w_o):
        B, Sq, M = x.shape[0], x.shape[1], x.shape[2]
        Sk = c_kv.shape[1]
        H, D = w_q.shape[1], w_q.shape[2]
        q = jnp.einsum("bqm,mhd->bhqd", x, w_q)
        k = jnp.einsum("bkc,chd->bhkd", c_kv, w_uk)
        v = jnp.einsum("bkc,chd->bhkd", c_kv, w_uv)
        scores = jnp.einsum("bhqd,bhkd->bhqk", q, k) * (D ** -0.5)
        off = Sk - Sq
        qi = jnp.arange(Sq)[:, None]
        kj = jnp.arange(Sk)[None, :]
        cmask = kj <= (qi + off)
        scores = jnp.where(cmask[None, None], scores, -1e9)
        p = _softmax(scores, axis=-1)
        ctx = jnp.einsum("bhqk,bhkd->bhqd", p, v)
        return jnp.einsum("bhqd,hdm->bqm", ctx, w_o)

    def _B_ref(x, w1, b1, w2, b2):
        h = jnp.einsum("bsd,df->bsf", x, w1) + b1
        h = _gelu(h)
        return jnp.einsum("bsf,fd->bsd", h, w2) + b2

    x = A_x
    xn = _layernorm(x, axis=-1)
    s = _A_ref(xn, A_c_kv, A_w_q, A_w_uk, A_w_uv, A_w_o)
    g = _silu(_B_ref(xn, B_w1, B_b1, B_w2, B_b2))
    return x + s * g
```

```python
import jax
import jax.numpy as jnp
from jax import lax
import jax.experimental.pallas as pl
import jax.experimental.pallas.tpu as pltpu

F32 = jnp.float32
BF16 = jnp.bfloat16

B, H, SK, D, M, DC, F = 2, 32, 16384, 128, 512, 512, 1792
LOG2E = 1.4426950408889634
NT = (((1,), (1,)), ((), ()))

NS = 32
CK = 2048
NC = B * SK // CK
RING = 4
NP = 13
LAST = 16
WO_BOUNDS = (12, 22, 28, 30, 31, NS)

I_WQ, I_WUK, I_C = 0, 2, 4
I_WUV = I_C + NC
I_W1, I_W2, I_WO = I_WUV + 1, I_WUV + 2, I_WUV + 3
I_X = I_WO + len(WO_BOUNDS) - 1


def _kernel(x_hbm, ckv_hbm, wq_hbm, wuk_hbm, wuv_hbm, wo_hbm, w1_hbm, b1_hbm, w2_hbm, b2_hbm,
            o_hbm,
            x_buf, b1_buf, b2_buf, c_buf, wq_buf, wuk_buf, wuv_buf, wo_buf, w1_buf, w2_buf, o_buf,
            gate_ref, xb, ring, t8, qa_ref, acc_ref, m_ref, l_ref, a_buf, ctx_ref, sems, sem_in, sem_out):
    def wait_filled(view, i):
        pltpu.make_async_copy(view, view, sems.at[i]).wait()

    def loop(lo, hi, f):
        lax.fori_loop(lo, hi, lambda i, _: f(i), None)

    def start_heads(hbm, buf, i, sem):
        pltpu.make_async_copy(hbm.at[:, pl.ds(i * 4, 4)], buf.at[:, pl.ds(i * 4, 4)], sems.at[sem]).start()

    def start_ckv(t):
        o = pl.multiple_of(t % NS * 32, 32)
        pltpu.make_async_copy(ckv_hbm.at[t // NS, :, pl.ds(o, 32)], c_buf.at[t // 4, pl.ds((t % 4) * 16, 16)],
                              sems.at[I_C + t // 4]).start()

    def wo_slot(k, r0=0, n=32):
        o = k * 32 + r0 if isinstance(k, int) else pl.multiple_of(k * 32 + r0, 32)
        return wo_hbm.at[:, pl.ds(o, n)], wo_buf.at[k, :, pl.ds(r0, n)]

    def relay(p, out):
        if isinstance(p, int) and p == NP - 1:
            (src, dst), mid = wo_slot(p, 0, LAST), ring.at[p % RING, :, pl.ds(0, LAST)]
        else:
            (src, dst), mid = wo_slot(p), ring.at[p % RING]
        if out:
            return pltpu.make_async_copy(mid, dst, sem_out.at[p % RING])
        return pltpu.make_async_copy(src, mid, sem_in.at[p % RING])

    def relay_step(p):
        dynamic = not isinstance(p, int)
        relay(p, False).wait()
        relay(p, True).start()
        if dynamic or p + 2 < NP:
            if dynamic or p + 2 >= RING:
                relay(p + 2 - RING, True).wait()
            relay(p + 2, False).start()

    small = [pltpu.make_async_copy(a, b, sems.at[I_X]) for a, b in ((x_hbm, x_buf), (b1_hbm, b1_buf), (b2_hbm, b2_buf))]
    start_heads(wq_hbm, wq_buf, 0, I_WQ)
    relay(0, False).start()
    relay(1, False).start()
    for cp in small:
        cp.start()
    loop(1, 24, lambda i: start_heads(wq_hbm, wq_buf, i, I_WQ + i // 16))

    for cp in small:
        cp.wait()
    x = x_buf[...].astype(F32)
    xc = x - jnp.mean(x, axis=-1, keepdims=True)
    var = jnp.mean(xc * xc, axis=-1, keepdims=True)
    xn = (xc * lax.rsqrt(var + 1e-5)).astype(BF16)
    for b in range(B):
        for j in range(M // 128):
            row = xn.astype(F32)[b:b + 1, j * 128:(j + 1) * 128]
            xb[b, pl.ds(j * 128, 128), :] = jnp.broadcast_to(row, (128, 128)).T

    q01 = (jnp.zeros((H, D), F32), jnp.zeros((H, D), F32))
    for j in range(2):
        wait_filled(wq_buf.at[:, pl.ds(64 * j, 64)], I_WQ + j)
        if j == 0:
            relay_step(0)
            loop(24, NS, lambda i: start_heads(wq_hbm, wq_buf, i, I_WQ + 1))
            loop(0, 8, lambda i: start_heads(wuk_hbm, wuk_buf, i, I_WUK))
        else:
            loop(8, 24, lambda i: start_heads(wuk_hbm, wuk_buf, i, I_WUK + i // 16))

        def q_body(i, carry, j=j):
            q0, q1 = carry
            n, r = i // 8, 64 * j + i % 8 * 8
            for u in range(8):
                w = wq_buf[n, r + u].astype(F32)
                q0 = q0 + xb[0, pl.ds(n * 128 + r + u, 1), :] * w
                q1 = q1 + xb[1, pl.ds(n * 128 + r + u, 1), :] * w
            return q0, q1

        q01 = lax.fori_loop(0, 32, q_body, q01)
    q = jnp.concatenate([q01[0], q01[1], jnp.zeros((128 - B * H, D), F32)], axis=0).astype(BF16)

    group = (lax.broadcasted_iota(jnp.int32, (16, 8, 128), 2) % H) // 8
    for j in range(2):
        wait_filled(wuk_buf.at[:, pl.ds(64 * j, 64)], I_WUK + j)
        if j == 0:
            relay_step(1)
            loop(24, NS, lambda i: start_heads(wuk_hbm, wuk_buf, i, I_WUK + 1))
            loop(0, 12, start_ckv)

        def qa_body(i, j=j):
            for s in range(2):
                r0 = 64 * j + (i % 2) * 32 + s * 16
                u = wuk_buf[i // 2, pl.ds(r0, 16)].reshape(16 * H, D)
                r = lax.dot_general(u, q, NT, preferred_element_type=F32).reshape(16, 4, 8, 128)
                v = jnp.where(group == 0, r[:, 0],
                              jnp.where(group == 1, r[:, 1], jnp.where(group == 2, r[:, 2], r[:, 3])))
                t8[pl.ds(pl.multiple_of((i // 2 * 128 + r0) * 8, 128), 128), :] = v.reshape(128, 128)

        loop(0, 8, qa_body)
    sub = lax.broadcasted_iota(jnp.int32, (128, 128), 1) % 8
    for j in range(DC // 128):
        t = t8[pl.ds(j * 1024, 128, stride=8), :]
        for s in range(1, 8):
            t = jnp.where(sub == s, t8[pl.ds(j * 1024 + s, 128, stride=8), :], t)
        qa_ref[:, j * 128:(j + 1) * 128] = (t.T[:B * H] * (D ** -0.5 * LOG2E)).astype(BF16)

    m_ref[...] = jnp.full((B * H, 128), -jnp.inf, F32)
    l_ref[...] = jnp.zeros((B * H, 128), F32)
    acc_ref[...] = jnp.zeros((B * H, DC), F32)

    def chunk(ci):
        wait_filled(c_buf.at[ci], I_C + ci)
        pl.when(ci % 2 == 0)(lambda: relay_step(2 + ci // 2))

        @pl.when(ci + 3 < NC)
        def _():
            for e in range(4):
                start_ckv((ci + 3) * 4 + e)

        @pl.when(ci >= NC - 2)
        def _():
            loop((ci - NC + 2) * 12, (ci - NC + 3) * 12, lambda i: start_heads(wuv_hbm, wuv_buf, i, I_WUV))

        hrows = pl.ds(pl.multiple_of(ci // (NC // B) * H, H), H)
        c = c_buf[ci].reshape(CK, DC)
        sc = lax.dot_general(qa_ref[hrows, :], c, NT, preferred_element_type=F32)
        m_prev = m_ref[hrows, :]
        m_new = jnp.maximum(m_prev, jnp.max(sc, axis=1, keepdims=True))
        p = jnp.exp2(sc - m_new[:, :1])
        alpha = jnp.exp2(m_prev - m_new)
        l_ref[hrows, :] = alpha * l_ref[hrows, :] + jnp.sum(p, axis=1, keepdims=True)
        m_ref[hrows, :] = m_new
        pv = jnp.dot(p.astype(BF16), c, preferred_element_type=F32)
        acc_ref[hrows, :] = acc_ref[hrows, :] * alpha[:, :1] + pv

    loop(0, NC, chunk)

    loop(24, NS, lambda i: start_heads(wuv_hbm, wuv_buf, i, I_WUV))
    pltpu.make_async_copy(w1_hbm, w1_buf, sems.at[I_W1]).start()
    pltpu.make_async_copy(w2_hbm, w2_buf, sems.at[I_W2]).start()
    pc = acc_ref[...] / l_ref[...][:, :1]
    lane = lax.broadcasted_iota(jnp.int32, (B * H, 128), 1)
    head = lax.broadcasted_iota(jnp.int32, (B * H, 128), 0) % H
    diag = (lane % H) == head
    for j in range(DC // 128):
        pcj = pc[:, j * 128:(j + 1) * 128]
        for t in range(32):
            rep = jnp.take_along_axis(pcj, lane // H + 4 * t, axis=1)
            a_buf[j, :, t * 128:(t + 1) * 128] = jnp.where(diag, rep, 0.0).astype(BF16)
    relay_step(10)
    wait_filled(wuv_buf, I_WUV)
    for j in range(len(WO_BOUNDS) - 1):
        for k in range(WO_BOUNDS[j], WO_BOUNDS[j + 1]):
            src, dst = wo_slot(k, LAST, 32 - LAST) if k == NP - 1 else wo_slot(k)
            pltpu.make_async_copy(src, dst, sems.at[I_WO + j]).start()

    def ctx_body(j, ctx):
        return ctx + jnp.dot(a_buf[j], wuv_buf[j].reshape(128 * H, D), preferred_element_type=F32)

    ctx = lax.fori_loop(0, DC // 128, ctx_body, jnp.zeros((B * H, D), F32))
    ctx_ref[...] = jnp.zeros_like(ctx_ref)
    for b in range(B):
        ctx_ref[pl.ds(b, H, stride=8), :] = ctx[b * H:(b + 1) * H]

    wait_filled(w1_buf, I_W1)
    relay_step(11)
    h = jnp.dot(xn, w1_buf[...], preferred_element_type=F32) + b1_buf[...].astype(F32).reshape(1, F)
    h = jax.nn.gelu(h, approximate=True).astype(BF16)
    wait_filled(w2_buf, I_W2)
    relay_step(12)
    gg = jnp.dot(h, w2_buf[...], preferred_element_type=F32) + b2_buf[...].astype(F32).reshape(1, M)
    gate_ref[...] = gg * jax.nn.sigmoid(gg)

    quarter = lax.broadcasted_iota(jnp.int32, (8, 128), 1) // 32

    def ctx_slots(k0, k1):
        tiles = []
        for k in range(k0, k1):
            out = None
            for t in range(4):
                a = ctx_ref[pl.ds((8 * t + k // 4) * 8, 8), :]
                if (t - k) % 4:
                    a = pltpu.roll(a, 32 * ((t - k) % 4), 1)
                out = a if out is None else jnp.where(quarter == t, a, out)
            tiles.append(out.astype(BF16))
        return jnp.concatenate(tiles, axis=1)

    def project(a, k0, k1):
        return jnp.dot(a, wo_buf[pl.ds(k0, k1 - k0)].reshape((k1 - k0) * 128, M), preferred_element_type=F32)

    for p in range(NP - RING, NP - 2):
        relay(p, True).wait()
    s = project(ctx_slots(0, NP - 2), 0, NP - 2)
    for j in range(len(WO_BOUNDS) - 1):
        k0, k1 = WO_BOUNDS[j], WO_BOUNDS[j + 1]
        if j == 0:
            k0 += 1
        if j == 1:
            relay(NP - 2, True).wait()
            relay(NP - 1, True).wait()
            s = s + project(ctx_slots(NP - 2, NP), NP - 2, NP)
        a = ctx_slots(k0, k1)
        wait_filled(wo_buf.at[pl.ds(k0, k1 - k0)], I_WO + j)
        if j == 0:
            wait_filled(wo_slot(NP - 1, LAST, 32 - LAST)[1], I_WO)
        s = s + project(a, k0, k1)
    for j in range(M // 128):
        cols = slice(j * 128, (j + 1) * 128)
        o_buf[:, cols] = (x_buf[:, cols].astype(F32) + s[:B, cols] * gate_ref[:, cols]).astype(BF16)
    out = pltpu.make_async_copy(o_buf, o_hbm, sems.at[I_X])
    out.start()
    out.wait()


@jax.jit
def pallas_recurrent_scan__compressed_kv_cla__dense_activation_gelu__decode_kernel(
    A_x: jax.Array,
    A_c_kv: jax.Array,
    A_w_q: jax.Array,
    A_w_uk: jax.Array,
    A_w_uv: jax.Array,
    A_w_o: jax.Array,
    B_x: jax.Array,
    B_w1: jax.Array,
    B_b1: jax.Array,
    B_w2: jax.Array,
    B_b2: jax.Array,
):
    del B_x
    out = pl.pallas_call(
        _kernel,
        out_shape=jax.ShapeDtypeStruct((B, M), BF16),
        in_specs=[pl.BlockSpec(memory_space=pltpu.HBM)] * 10,
        out_specs=pl.BlockSpec(memory_space=pltpu.HBM),
        scratch_shapes=[
            pltpu.VMEM((B, M), BF16), pltpu.VMEM((F,), BF16), pltpu.VMEM((M,), BF16),
            pltpu.VMEM((NC, CK // 32, 32, DC), BF16),
            pltpu.VMEM((4, 128, H, D), BF16), pltpu.VMEM((4, 128, H, D), BF16), pltpu.VMEM((4, 128, H, D), BF16),
            pltpu.VMEM((NS, 4, 32, M), BF16), pltpu.VMEM((M, F), BF16), pltpu.VMEM((F, M), BF16),
            pltpu.VMEM((B, M), BF16),
            pltpu.VMEM((B, M), F32), pltpu.VMEM((B, M, 128), F32),
            pltpu.SMEM((RING, 4, 32, M), BF16),
            pltpu.VMEM((DC * 8 + 8, 128), F32),
            pltpu.VMEM((B * H, DC), BF16), pltpu.VMEM((B * H, DC), F32),
            pltpu.VMEM((B * H, 128), F32), pltpu.VMEM((B * H, 128), F32),
            pltpu.VMEM((DC // 128, B * H, 128 * H), BF16),
            pltpu.VMEM((H * 8, D), F32),
            pltpu.SemaphoreType.DMA((I_X + 1,)), pltpu.SemaphoreType.DMA((RING,)), pltpu.SemaphoreType.DMA((RING,)),
        ],
        compiler_params=pltpu.CompilerParams(vmem_limit_bytes=100 * 1024 * 1024,
                                             disable_bounds_checks=True, disable_semaphore_checks=True),
    )(A_x.reshape(B, M), A_c_kv.reshape(B, 16, 1024, DC), A_w_q.reshape(4, 128, H, D), A_w_uk.reshape(4, 128, H, D),
      A_w_uv.reshape(4, 128, H, D), A_w_o.reshape(4, 1024, M), B_w1, B_b1, B_w2, B_b2)
    return out.reshape(B, 1, M)
```

```python
import jax
import jax.numpy as jnp
from jax import lax
import jax.experimental.pallas as pl
import jax.experimental.pallas.tpu as pltpu

F32 = jnp.float32
BF16 = jnp.bfloat16

B, H, SK, D, M, DC, F = 2, 32, 16384, 128, 512, 512, 1792
LOG2E = 1.4426950408889634
NT = (((1,), (1,)), ((), ()))

NS = 32
CK = 2048
NC = B * SK // CK

RING = 3
NP = 13
WO_SLOTS = ((3, 6), (6, 7), (7, 8))
WO_MXU = ((3, 5), (5, 6))
WO_VPU = (72, 128, 192, 224, 240, 256)
V0 = WO_MXU[-1][1]

I_WQ, I_WUK, I_C = 0, 2, 4
I_WUV = I_C + NC
I_W1, I_W2, I_SLOTS = I_WUV + 1, I_WUV + 2, I_WUV + 3
I_MXU = I_SLOTS + len(WO_SLOTS)
I_VPU = I_MXU + len(WO_MXU)
I_X = I_VPU + len(WO_VPU) - 1


def _kernel(x_hbm, ckv_hbm, wq_hbm, wuk_hbm, wuv_hbm, wo_hbm, w1_hbm, b1_hbm, w2_hbm, b2_hbm,
            o_hbm,
            x_buf, b1_buf, b2_buf, c_buf, wq_buf, wuk_buf, wuv_buf, wo_buf, w1_buf, w2_buf, o_buf,
            xf_ref, gate_ref, bc_ref, ring, t8, qa_ref, acc_ref, m_ref, l_ref, a_buf, ctx_ref, sems, sem_in, sem_out):
    def wait_filled(view, i):
        pltpu.make_async_copy(view, view, sems.at[i]).wait()

    def loop(lo, hi, f):
        lax.fori_loop(lo, hi, lambda i, _: f(i), None)

    def start_heads(hbm, buf, i, sem):
        pltpu.make_async_copy(hbm.at[:, pl.ds(i * 4, 4)], buf.at[:, pl.ds(i * 4, 4)], sems.at[sem]).start()

    def start_ckv(t):
        o = pl.multiple_of(t % NS * 32, 32)
        pltpu.make_async_copy(ckv_hbm.at[t // NS, :, pl.ds(o, 32)], c_buf.at[t // 4, pl.ds((t % 4) * 16, 16)],
                              sems.at[I_C + t // 4]).start()

    def wo_rows(blk, o, n):
        return wo_hbm.at[blk, pl.ds(o, n)], wo_buf.at[blk, pl.ds(o, n)]

    def relay(p, out):
        if isinstance(p, int) and p == NP - 1:
            (src, dst), mid = wo_rows(3, V0 * D, WO_VPU[0]), ring.at[p % RING, pl.ds(0, WO_VPU[0])]
        else:
            o = p // 4 * D if isinstance(p, int) else pl.multiple_of(p // 4 * D, D)
            (src, dst), mid = wo_rows(p % 4, o, D), ring.at[p % RING]
        if out:
            return pltpu.make_async_copy(mid, dst, sem_out.at[p % RING])
        return pltpu.make_async_copy(src, mid, sem_in.at[p % RING])

    def relay_step(p):
        dynamic = not isinstance(p, int)
        relay(p, False).wait()
        relay(p, True).start()
        if dynamic or p + 2 < NP:
            if dynamic or p + 2 >= RING:
                relay(p + 2 - RING, True).wait()
            relay(p + 2, False).start(priority=1)

    def broadcast_rows(v, o):
        for b in range(B):
            bc_ref[b, pl.ds(o, 128), :] = jnp.broadcast_to(v[b:b + 1], (128, 128)).T

    small = [pltpu.make_async_copy(a, b, sems.at[I_X]) for a, b in ((x_hbm, x_buf), (b1_hbm, b1_buf), (b2_hbm, b2_buf))]
    for n in range(4):
        pltpu.make_async_copy(wq_hbm.at[n, pl.ds(0, 32)], wq_buf.at[n, pl.ds(0, 32)], sems.at[I_WQ]).start()
        if n < 2:
            relay(n, False).start(priority=1)
        if n == 0:
            for cp in small:
                cp.start()
    loop(8, 24, lambda i: start_heads(wq_hbm, wq_buf, i, I_WQ + i // 16))

    for cp in small:
        cp.wait()
    x = x_buf[...].astype(F32)
    xc = x - jnp.mean(x, axis=-1, keepdims=True)
    var = jnp.mean(xc * xc, axis=-1, keepdims=True)
    xn = (xc * lax.rsqrt(var + 1e-5)).astype(BF16)
    for j in range(M // 128):
        broadcast_rows(xn.astype(F32)[:, j * 128:(j + 1) * 128], j * 128)
        xf_ref[j] = x_buf[:, j * 128:(j + 1) * 128].astype(F32)

    q01 = (jnp.zeros((H, D), F32), jnp.zeros((H, D), F32))
    for j in range(2):
        wait_filled(wq_buf.at[:, pl.ds(64 * j, 64)], I_WQ + j)
        if j == 0:
            relay_step(0)
            loop(24, NS, lambda i: start_heads(wq_hbm, wq_buf, i, I_WQ + 1))
            loop(0, 8, lambda i: start_heads(wuk_hbm, wuk_buf, i, I_WUK))
        else:
            loop(8, 24, lambda i: start_heads(wuk_hbm, wuk_buf, i, I_WUK + i // 16))

        def q_body(i, carry, j=j):
            q0, q1 = carry
            n, r = i // 8, 64 * j + i % 8 * 8
            for u in range(8):
                w = wq_buf[n, r + u].astype(F32)
                q0 = q0 + bc_ref[0, pl.ds(n * 128 + r + u, 1), :] * w
                q1 = q1 + bc_ref[1, pl.ds(n * 128 + r + u, 1), :] * w
            return q0, q1

        q01 = lax.fori_loop(0, 32, q_body, q01)
    q = jnp.concatenate([q01[0], q01[1], jnp.zeros((128 - B * H, D), F32)], axis=0).astype(BF16)

    group = (lax.broadcasted_iota(jnp.int32, (16, 8, 128), 2) % H) // 8
    for j in range(2):
        wait_filled(wuk_buf.at[:, pl.ds(64 * j, 64)], I_WUK + j)
        if j == 0:
            relay_step(1)
            loop(24, NS, lambda i: start_heads(wuk_hbm, wuk_buf, i, I_WUK + 1))
            loop(0, 12, start_ckv)

        def qa_body(i, j=j):
            for s in range(2):
                r0 = 64 * j + (i % 2) * 32 + s * 16
                u = wuk_buf[i // 2, pl.ds(r0, 16)].reshape(16 * H, D)
                r = lax.dot_general(u, q, NT, preferred_element_type=F32).reshape(16, 4, 8, 128)
                v = jnp.where(group == 0, r[:, 0],
                              jnp.where(group == 1, r[:, 1], jnp.where(group == 2, r[:, 2], r[:, 3])))
                t8[pl.ds(pl.multiple_of((i // 2 * 128 + r0) * 8, 128), 128), :] = v.reshape(128, 128)

        loop(0, 8, qa_body)
    sub = lax.broadcasted_iota(jnp.int32, (128, 128), 1) % 8
    for j in range(DC // 128):
        t = t8[pl.ds(j * 1024, 128, stride=8), :]
        for s in range(1, 8):
            t = jnp.where(sub == s, t8[pl.ds(j * 1024 + s, 128, stride=8), :], t)
        qa_ref[:, j * 128:(j + 1) * 128] = (t.T[:B * H] * (D ** -0.5 * LOG2E)).astype(BF16)

    m_ref[...] = jnp.full((B * H, 128), -jnp.inf, F32)
    l_ref[...] = jnp.zeros((B * H, 128), F32)
    acc_ref[...] = jnp.zeros((B * H, DC), F32)

    def chunk(ci):
        wait_filled(c_buf.at[ci], I_C + ci)
        pl.when(ci % 2 == 0)(lambda: relay_step(2 + ci // 2))

        @pl.when(ci + 3 < NC)
        def _():
            for e in range(4):
                start_ckv((ci + 3) * 4 + e)

        @pl.when(ci >= NC - 2)
        def _():
            loop((ci - NC + 2) * 12, (ci - NC + 3) * 12, lambda i: start_heads(wuv_hbm, wuv_buf, i, I_WUV))

        hrows = pl.ds(pl.multiple_of(ci // (NC // B) * H, H), H)
        c = c_buf[ci].reshape(CK, DC)
        sc = lax.dot_general(qa_ref[hrows, :], c, NT, preferred_element_type=F32)
        m_prev = m_ref[hrows, :]
        m_new = jnp.maximum(m_prev, jnp.max(sc, axis=1, keepdims=True))
        p = jnp.exp2(sc - m_new[:, :1])
        alpha = jnp.exp2(m_prev - m_new)
        l_ref[hrows, :] = alpha * l_ref[hrows, :] + jnp.sum(p, axis=1, keepdims=True)
        m_ref[hrows, :] = m_new
        pv = jnp.dot(p.astype(BF16), c, preferred_element_type=F32)
        acc_ref[hrows, :] = acc_ref[hrows, :] * alpha[:, :1] + pv

    loop(0, NC, chunk)

    loop(24, NS, lambda i: start_heads(wuv_hbm, wuv_buf, i, I_WUV))
    w1_copy = pltpu.make_async_copy(w1_hbm, w1_buf, sems.at[I_W1])
    w2_copy = pltpu.make_async_copy(w2_hbm, w2_buf, sems.at[I_W2])
    w1_copy.start()
    w2_copy.start()
    pc = acc_ref[...] / l_ref[...][:, :1]
    lane = lax.broadcasted_iota(jnp.int32, (B * H, 128), 1)
    head = lax.broadcasted_iota(jnp.int32, (B * H, 128), 0) % H
    diag = (lane % H) == head
    for j in range(DC // 128):
        pcj = pc[:, j * 128:(j + 1) * 128]
        for t in range(32):
            rep = jnp.take_along_axis(pcj, lane // H + 4 * t, axis=1)
            a_buf[j, :, t * 128:(t + 1) * 128] = jnp.where(diag, rep, 0.0).astype(BF16)
    relay_step(10)
    wait_filled(wuv_buf, I_WUV)

    for j, (g0, g1) in enumerate(WO_SLOTS):
        def start_slot(k, j=j):
            pltpu.make_async_copy(*wo_rows(pl.ds(0, 3), pl.multiple_of(k * 32, 32), 32), sems.at[I_SLOTS + j]).start()

        loop(4 * g0, 4 * g1, start_slot)
    mxu_copies = [pltpu.make_async_copy(*wo_rows(3, g0 * D, (g1 - g0) * D), sems.at[I_MXU + j])
                  for j, (g0, g1) in enumerate(WO_MXU)]
    vpu_copies = [pltpu.make_async_copy(*wo_rows(3, V0 * D + lo, hi - lo), sems.at[I_VPU + j])
                  for j, (lo, hi) in enumerate(zip(WO_VPU[:-1], WO_VPU[1:]))]
    for cp in mxu_copies:
        cp.start()

    def ctx_body(j, ctx):
        return ctx + jnp.dot(a_buf[j], wuv_buf[j].reshape(128 * H, D), preferred_element_type=F32)

    ctx = lax.fori_loop(0, DC // 128, ctx_body, jnp.zeros((B * H, D), F32))
    ctx_ref[...] = jnp.zeros_like(ctx_ref)
    for b in range(B):
        ctx_ref[pl.ds(b, H, stride=8), :] = ctx[b * H:(b + 1) * H]

    w1_copy.wait()
    relay_step(11)
    h = jnp.dot(xn, w1_buf[...], preferred_element_type=F32) + b1_buf[...].astype(F32).reshape(1, F)
    h = jax.nn.gelu(h, approximate=True).astype(BF16)
    w2_copy.wait()
    relay_step(12)
    for cp in vpu_copies:
        cp.start()
    gg = jnp.dot(h, w2_buf[...], preferred_element_type=F32) + b2_buf[...].astype(F32).reshape(1, M)
    gate_ref[...] = gg * jax.nn.sigmoid(gg)

    def ctx_heads(h0, h1):
        return jnp.concatenate([ctx_ref[pl.ds(8 * k, 8), :] for k in range(h0, h1)], axis=1).astype(BF16)

    def project(s, blocks, g0, g1):
        for t in blocks:
            s = s + jnp.dot(ctx_heads(8 * t + g0, 8 * t + g1), wo_buf[t, pl.ds(g0 * D, (g1 - g0) * D), :],
                            preferred_element_type=F32)
        return s

    for g in range(V0, 8):
        broadcast_rows(ctx_heads(24 + g, 25 + g).astype(F32), (g - V0) * D)
    s = project(jnp.zeros((8, M), F32), range(4), 0, 2)
    for j, (g0, g1) in enumerate(WO_SLOTS):
        if j == 1:
            for p in range(NP - RING, NP - 1):
                relay(p, True).wait()
            s = project(s, range(4), 2, 3)
        wait_filled(wo_rows(pl.ds(0, 3), g0 * D, (g1 - g0) * D)[1], I_SLOTS + j)
        s = project(s, range(3), g0, g1)
    for cp, (g0, g1) in zip(mxu_copies, WO_MXU):
        cp.wait()
        s = project(s, [3], g0, g1)
    sub = lax.broadcasted_iota(jnp.int32, (8, 128), 0)
    acc = [[jnp.where(sub == b, s[:, j * 128:(j + 1) * 128], 0.0) for b in range(B)] for j in range(M // 128)]
    for cp, lo, hi in zip([relay(NP - 1, True)] + vpu_copies, (0,) + WO_VPU[:-1], WO_VPU):
        cp.wait()
        for r in range(lo, hi, 8):
            cb = [bc_ref[b, pl.ds(r, 8), :] for b in range(B)]
            for j in range(M // 128):
                w = wo_buf[3, pl.ds(V0 * D + r, 8), pl.ds(j * 128, 128)].astype(F32)
                for b in range(B):
                    acc[j][b] = acc[j][b] + w * cb[b]
    even = (sub & 1) == 0
    for j in range(M // 128):
        cols = slice(j * 128, (j + 1) * 128)
        t = jnp.where(even, acc[j][0], acc[j][1]) + pltpu.roll(jnp.where(even, acc[j][1], acc[j][0]), 7, 0)
        t = t + pltpu.roll(t, 2, 0)
        t = t + pltpu.roll(t, 4, 0)
        o_buf[:, cols] = (xf_ref[j] + t[:B] * gate_ref[:, cols]).astype(BF16)
    out = pltpu.make_async_copy(o_buf, o_hbm, sems.at[I_X])
    out.start()
    out.wait()


@jax.jit
def pallas_recurrent_scan__compressed_kv_cla__dense_activation_gelu__decode_kernel(
    A_x: jax.Array,
    A_c_kv: jax.Array,
    A_w_q: jax.Array,
    A_w_uk: jax.Array,
    A_w_uv: jax.Array,
    A_w_o: jax.Array,
    B_x: jax.Array,
    B_w1: jax.Array,
    B_b1: jax.Array,
    B_w2: jax.Array,
    B_b2: jax.Array,
):
    del B_x
    out = pl.pallas_call(
        _kernel,
        out_shape=jax.ShapeDtypeStruct((B, M), BF16),
        in_specs=[pl.BlockSpec(memory_space=pltpu.HBM)] * 10,
        out_specs=pl.BlockSpec(memory_space=pltpu.HBM),
        scratch_shapes=[
            pltpu.VMEM((B, M), BF16), pltpu.VMEM((F,), BF16), pltpu.VMEM((M,), BF16),
            pltpu.VMEM((NC, CK // 32, 32, DC), BF16),
            pltpu.VMEM((4, 128, H, D), BF16), pltpu.VMEM((4, 128, H, D), BF16), pltpu.VMEM((4, 128, H, D), BF16),
            pltpu.VMEM((4, 8 * D, M), BF16), pltpu.VMEM((M, F), BF16), pltpu.VMEM((F, M), BF16),
            pltpu.VMEM((B, M), BF16),
            pltpu.VMEM((M // 128, B, 128), F32), pltpu.VMEM((B, M), F32), pltpu.VMEM((B, M, 128), F32),
            pltpu.SMEM((RING, D, M), BF16),
            pltpu.VMEM((DC * 8 + 8, 128), F32),
            pltpu.VMEM((B * H, DC), BF16), pltpu.VMEM((B * H, DC), F32),
            pltpu.VMEM((B * H, 128), F32), pltpu.VMEM((B * H, 128), F32),
            pltpu.VMEM((DC // 128, B * H, 128 * H), BF16),
            pltpu.VMEM((H * 8 + 8, D), F32),
            pltpu.SemaphoreType.DMA((I_X + 1,)), pltpu.SemaphoreType.DMA((RING,)), pltpu.SemaphoreType.DMA((RING,)),
        ],
        compiler_params=pltpu.CompilerParams(vmem_limit_bytes=100 * 1024 * 1024,
                                             disable_bounds_checks=True, disable_semaphore_checks=True),
    )(A_x.reshape(B, M), A_c_kv.reshape(B, 16, 1024, DC), A_w_q.reshape(4, 128, H, D), A_w_uk.reshape(4, 128, H, D),
      A_w_uv.reshape(4, 128, H, D), A_w_o.reshape(4, 8 * D, M), B_w1, B_b1, B_w2, B_b2)
    return out.reshape(B, 1, M)
```

```python
import jax
import jax.numpy as jnp
from jax import lax
import jax.experimental.pallas as pl
import jax.experimental.pallas.tpu as pltpu

F32 = jnp.float32
BF16 = jnp.bfloat16

B, H, SK, D, M, DC, F = 2, 32, 16384, 128, 512, 512, 1792
LOG2E = 1.4426950408889634
NT = (((1,), (1,)), ((), ()))

NS = 32
CK = 2048
NC = B * SK // CK

RING = 3
NP = 13
WO_SLOTS = ((3, 7), (7, 8))
LAST0 = 3 * D
WO_LAST = (72, 256, 384, 432, 480, 520, 552, 584, 608, 624, 640)

I_WQ, I_WUK, I_C = 0, 2, 4
I_WUV = I_C + NC
I_W1, I_W2, I_SLOTS = I_WUV + 1, I_WUV + 2, I_WUV + 3
I_LAST = I_SLOTS + len(WO_SLOTS)
I_X = I_LAST + len(WO_LAST) - 1


def _kernel(x_hbm, ckv_hbm, wq_hbm, wuk_hbm, wuv_hbm, wo_hbm, w1_hbm, b1_hbm, w2_hbm, b2_hbm,
            o_hbm,
            x_buf, b1_buf, b2_buf, c_buf, wq_buf, wuk_buf, wuv_buf, wo_buf, w1_buf, w2_buf, o_buf,
            xf_ref, gate_ref, bc_ref, ring, t8, qa_ref, acc_ref, m_ref, l_ref, a_buf, ctx_ref, sems, sem_in, sem_out):
    def wait_filled(view, i):
        pltpu.make_async_copy(view, view, sems.at[i]).wait()

    def loop(lo, hi, f):
        lax.fori_loop(lo, hi, lambda i, _: f(i), None)

    def start_heads(hbm, buf, i, sem):
        pltpu.make_async_copy(hbm.at[:, pl.ds(i * 4, 4)], buf.at[:, pl.ds(i * 4, 4)], sems.at[sem]).start()

    def start_ckv(t):
        o = pl.multiple_of(t % NS * 32, 32)
        pltpu.make_async_copy(ckv_hbm.at[t // NS, :, pl.ds(o, 32)], c_buf.at[t // 4, pl.ds((t % 4) * 16, 16)],
                              sems.at[I_C + t // 4]).start()

    def wo_rows(blk, o, n):
        return wo_hbm.at[blk, pl.ds(o, n)], wo_buf.at[blk, pl.ds(o, n)]

    def relay(p, out):
        if isinstance(p, int) and p == NP - 1:
            (src, dst), mid = wo_rows(3, LAST0, WO_LAST[0]), ring.at[p % RING, pl.ds(0, WO_LAST[0])]
        else:
            o = p // 4 * D if isinstance(p, int) else pl.multiple_of(p // 4 * D, D)
            (src, dst), mid = wo_rows(p % 4, o, D), ring.at[p % RING]
        if out:
            return pltpu.make_async_copy(mid, dst, sem_out.at[p % RING])
        return pltpu.make_async_copy(src, mid, sem_in.at[p % RING])

    def relay_step(p):
        dynamic = not isinstance(p, int)
        relay(p, False).wait()
        relay(p, True).start()
        if dynamic or p + 2 < NP:
            if dynamic or p + 2 >= RING:
                relay(p + 2 - RING, True).wait()
            relay(p + 2, False).start(priority=1)

    def broadcast_rows(v, o):
        for b in range(B):
            bc_ref[b, pl.ds(o, 128), :] = jnp.broadcast_to(v[b:b + 1], (128, 128)).T

    small = [pltpu.make_async_copy(a, b, sems.at[I_X]) for a, b in ((x_hbm, x_buf), (b1_hbm, b1_buf), (b2_hbm, b2_buf))]
    for n in range(4):
        pltpu.make_async_copy(wq_hbm.at[n, pl.ds(0, 32)], wq_buf.at[n, pl.ds(0, 32)], sems.at[I_WQ]).start()
        if n < 2:
            relay(n, False).start(priority=1)
        if n == 0:
            for cp in small:
                cp.start()
    loop(8, 24, lambda i: start_heads(wq_hbm, wq_buf, i, I_WQ + i // 16))

    for cp in small:
        cp.wait()
    x = x_buf[...].astype(F32)
    xc = x - jnp.mean(x, axis=-1, keepdims=True)
    var = jnp.mean(xc * xc, axis=-1, keepdims=True)
    xn = (xc * lax.rsqrt(var + 1e-5)).astype(BF16)
    for j in range(M // 128):
        broadcast_rows(xn.astype(F32)[:, j * 128:(j + 1) * 128], j * 128)
        xf_ref[j] = x_buf[:, j * 128:(j + 1) * 128].astype(F32)

    q01 = (jnp.zeros((H, D), F32), jnp.zeros((H, D), F32))
    for j in range(2):
        wait_filled(wq_buf.at[:, pl.ds(64 * j, 64)], I_WQ + j)
        if j == 0:
            relay_step(0)
            loop(24, NS, lambda i: start_heads(wq_hbm, wq_buf, i, I_WQ + 1))
            loop(0, 8, lambda i: start_heads(wuk_hbm, wuk_buf, i, I_WUK))
        else:
            loop(8, 24, lambda i: start_heads(wuk_hbm, wuk_buf, i, I_WUK + i // 16))

        def q_body(i, carry, j=j):
            q0, q1 = carry
            n, r = i // 8, 64 * j + i % 8 * 8
            for u in range(8):
                w = wq_buf[n, r + u].astype(F32)
                q0 = q0 + bc_ref[0, pl.ds(n * 128 + r + u, 1), :] * w
                q1 = q1 + bc_ref[1, pl.ds(n * 128 + r + u, 1), :] * w
            return q0, q1

        q01 = lax.fori_loop(0, 32, q_body, q01)
    q = jnp.concatenate([q01[0], q01[1], jnp.zeros((128 - B * H, D), F32)], axis=0).astype(BF16)

    group = (lax.broadcasted_iota(jnp.int32, (16, 8, 128), 2) % H) // 8
    for j in range(2):
        wait_filled(wuk_buf.at[:, pl.ds(64 * j, 64)], I_WUK + j)
        if j == 0:
            relay_step(1)
            loop(24, NS, lambda i: start_heads(wuk_hbm, wuk_buf, i, I_WUK + 1))
            loop(0, 12, start_ckv)

        def qa_body(i, j=j):
            for s in range(2):
                r0 = 64 * j + (i % 2) * 32 + s * 16
                u = wuk_buf[i // 2, pl.ds(r0, 16)].reshape(16 * H, D)
                r = lax.dot_general(u, q, NT, preferred_element_type=F32).reshape(16, 4, 8, 128)
                v = jnp.where(group == 0, r[:, 0],
                              jnp.where(group == 1, r[:, 1], jnp.where(group == 2, r[:, 2], r[:, 3])))
                t8[pl.ds(pl.multiple_of((i // 2 * 128 + r0) * 8, 128), 128), :] = v.reshape(128, 128)

        loop(0, 8, qa_body)
    sub = lax.broadcasted_iota(jnp.int32, (128, 128), 1) % 8
    for j in range(DC // 128):
        t = t8[pl.ds(j * 1024, 128, stride=8), :]
        for s in range(1, 8):
            t = jnp.where(sub == s, t8[pl.ds(j * 1024 + s, 128, stride=8), :], t)
        qa_ref[:, j * 128:(j + 1) * 128] = (t.T[:B * H] * (D ** -0.5 * LOG2E)).astype(BF16)

    m_ref[...] = jnp.full((B * H, 128), -jnp.inf, F32)
    l_ref[...] = jnp.zeros((B * H, 128), F32)
    acc_ref[...] = jnp.zeros((B * H, DC), F32)

    def chunk(ci):
        wait_filled(c_buf.at[ci], I_C + ci)
        pl.when(ci % 2 == 0)(lambda: relay_step(2 + ci // 2))

        @pl.when(ci + 3 < NC)
        def _():
            for e in range(4):
                start_ckv((ci + 3) * 4 + e)

        @pl.when(ci >= NC - 2)
        def _():
            loop((ci - NC + 2) * 12, (ci - NC + 3) * 12, lambda i: start_heads(wuv_hbm, wuv_buf, i, I_WUV))

        hrows = pl.ds(pl.multiple_of(ci // (NC // B) * H, H), H)
        c = c_buf[ci].reshape(CK, DC)
        sc = lax.dot_general(qa_ref[hrows, :], c, NT, preferred_element_type=F32)
        m_prev = m_ref[hrows, :]
        m_new = jnp.maximum(m_prev, jnp.max(sc, axis=1, keepdims=True))
        p = jnp.exp2(sc - m_new[:, :1])
        alpha = jnp.exp2(m_prev - m_new)
        l_ref[hrows, :] = alpha * l_ref[hrows, :] + jnp.sum(p, axis=1, keepdims=True)
        m_ref[hrows, :] = m_new
        pv = jnp.dot(p.astype(BF16), c, preferred_element_type=F32)
        acc_ref[hrows, :] = acc_ref[hrows, :] * alpha[:, :1] + pv

    loop(0, NC, chunk)

    loop(24, NS, lambda i: start_heads(wuv_hbm, wuv_buf, i, I_WUV))
    w1_copy = pltpu.make_async_copy(w1_hbm, w1_buf, sems.at[I_W1])
    w2_copy = pltpu.make_async_copy(w2_hbm, w2_buf, sems.at[I_W2])
    w1_copy.start()
    w2_copy.start()
    pc = acc_ref[...] / l_ref[...][:, :1]
    lane = lax.broadcasted_iota(jnp.int32, (B * H, 128), 1)
    head = lax.broadcasted_iota(jnp.int32, (B * H, 128), 0) % H
    diag = (lane % H) == head
    for j in range(DC // 128):
        pcj = pc[:, j * 128:(j + 1) * 128]
        for t in range(32):
            rep = jnp.take_along_axis(pcj, lane // H + 4 * t, axis=1)
            a_buf[j, :, t * 128:(t + 1) * 128] = jnp.where(diag, rep, 0.0).astype(BF16)
    relay_step(10)
    wait_filled(wuv_buf, I_WUV)

    for j, (g0, g1) in enumerate(WO_SLOTS):
        def start_slot(k, j=j):
            pltpu.make_async_copy(*wo_rows(pl.ds(0, 3), pl.multiple_of(k * 32, 32), 32), sems.at[I_SLOTS + j]).start()

        loop(4 * g0, 4 * g1, start_slot)
    last = [(pltpu.make_async_copy(*wo_rows(3, LAST0 + lo, hi - lo), sems.at[I_LAST + j]), lo, hi)
            for j, (lo, hi) in enumerate(zip(WO_LAST[:-1], WO_LAST[1:]))]

    def ctx_body(j, ctx):
        return ctx + jnp.dot(a_buf[j], wuv_buf[j].reshape(128 * H, D), preferred_element_type=F32)

    ctx = lax.fori_loop(0, DC // 128, ctx_body, jnp.zeros((B * H, D), F32))
    ctx_ref[...] = jnp.zeros_like(ctx_ref)
    for b in range(B):
        ctx_ref[pl.ds(b, H, stride=8), :] = ctx[b * H:(b + 1) * H]

    w1_copy.wait()
    relay_step(11)
    h = jnp.dot(xn, w1_buf[...], preferred_element_type=F32) + b1_buf[...].astype(F32).reshape(1, F)
    h = jax.nn.gelu(h, approximate=True).astype(BF16)
    w2_copy.wait()
    relay_step(12)
    for cp, _, _ in last:
        cp.start()
    gg = jnp.dot(h, w2_buf[...], preferred_element_type=F32) + b2_buf[...].astype(F32).reshape(1, M)
    gate_ref[...] = gg * jax.nn.sigmoid(gg)

    def ctx_heads(h0, h1):
        return jnp.concatenate([ctx_ref[pl.ds(8 * k, 8), :] for k in range(h0, h1)], axis=1).astype(BF16)

    def project(s, blocks, g0, g1):
        for t in blocks:
            s = s + jnp.dot(ctx_heads(8 * t + g0, 8 * t + g1), wo_buf[t, pl.ds(g0 * D, (g1 - g0) * D), :],
                            preferred_element_type=F32)
        return s

    for g in range(3, 8):
        broadcast_rows(ctx_heads(24 + g, 25 + g).astype(F32), g * D - LAST0)
    s = project(jnp.zeros((8, M), F32), range(4), 0, 2)
    for j, (g0, g1) in enumerate(WO_SLOTS):
        if j == 1:
            for p in range(NP - RING, NP - 1):
                relay(p, True).wait()
            s = project(s, range(4), 2, 3)
        wait_filled(wo_rows(pl.ds(0, 3), g0 * D, (g1 - g0) * D)[1], I_SLOTS + j)
        s = project(s, range(3), g0, g1)
    sub = lax.broadcasted_iota(jnp.int32, (8, 128), 0)
    acc = [[jnp.where(sub == b, s[:, j * 128:(j + 1) * 128], 0.0) for b in range(B)] for j in range(M // 128)]
    for cp, lo, hi in last[:2] + [(relay(NP - 1, True), 0, WO_LAST[0])] + last[2:]:
        cp.wait()
        for r in range(lo, hi, 8):
            cb = [bc_ref[b, pl.ds(r, 8), :] for b in range(B)]
            for j in range(M // 128):
                w = wo_buf[3, pl.ds(LAST0 + r, 8), pl.ds(j * 128, 128)].astype(F32)
                for b in range(B):
                    acc[j][b] = acc[j][b] + w * cb[b]
    even = (sub & 1) == 0
    for j in range(M // 128):
        cols = slice(j * 128, (j + 1) * 128)
        t = jnp.where(even, acc[j][0], acc[j][1]) + pltpu.roll(jnp.where(even, acc[j][1], acc[j][0]), 7, 0)
        t = t + pltpu.roll(t, 2, 0)
        t = t + pltpu.roll(t, 4, 0)
        o_buf[:, cols] = (xf_ref[j] + t[:B] * gate_ref[:, cols]).astype(BF16)
    out = pltpu.make_async_copy(o_buf, o_hbm, sems.at[I_X])
    out.start()
    out.wait()


@jax.jit
def pallas_recurrent_scan__compressed_kv_cla__dense_activation_gelu__decode_kernel(
    A_x: jax.Array,
    A_c_kv: jax.Array,
    A_w_q: jax.Array,
    A_w_uk: jax.Array,
    A_w_uv: jax.Array,
    A_w_o: jax.Array,
    B_x: jax.Array,
    B_w1: jax.Array,
    B_b1: jax.Array,
    B_w2: jax.Array,
    B_b2: jax.Array,
):
    del B_x
    out = pl.pallas_call(
        _kernel,
        out_shape=jax.ShapeDtypeStruct((B, M), BF16),
        in_specs=[pl.BlockSpec(memory_space=pltpu.HBM)] * 10,
        out_specs=pl.BlockSpec(memory_space=pltpu.HBM),
        scratch_shapes=[
            pltpu.VMEM((B, M), BF16), pltpu.VMEM((F,), BF16), pltpu.VMEM((M,), BF16),
            pltpu.VMEM((NC, CK // 32, 32, DC), BF16),
            pltpu.VMEM((4, 128, H, D), BF16), pltpu.VMEM((4, 128, H, D), BF16), pltpu.VMEM((4, 128, H, D), BF16),
            pltpu.VMEM((4, 8 * D, M), BF16), pltpu.VMEM((M, F), BF16), pltpu.VMEM((F, M), BF16),
            pltpu.VMEM((B, M), BF16),
            pltpu.VMEM((M // 128, B, 128), F32), pltpu.VMEM((B, M), F32), pltpu.VMEM((B, WO_LAST[-1], 128), F32),
            pltpu.SMEM((RING, D, M), BF16),
            pltpu.VMEM((DC * 8 + 8, 128), F32),
            pltpu.VMEM((B * H, DC), BF16), pltpu.VMEM((B * H, DC), F32),
            pltpu.VMEM((B * H, 128), F32), pltpu.VMEM((B * H, 128), F32),
            pltpu.VMEM((DC // 128, B * H, 128 * H), BF16),
            pltpu.VMEM((H * 8 + 8, D), F32),
            pltpu.SemaphoreType.DMA((I_X + 1,)), pltpu.SemaphoreType.DMA((RING,)), pltpu.SemaphoreType.DMA((RING,)),
        ],
        compiler_params=pltpu.CompilerParams(vmem_limit_bytes=100 * 1024 * 1024,
                                             disable_bounds_checks=True, disable_semaphore_checks=True),
    )(A_x.reshape(B, M), A_c_kv.reshape(B, 16, 1024, DC), A_w_q.reshape(4, 128, H, D), A_w_uk.reshape(4, 128, H, D),
      A_w_uv.reshape(4, 128, H, D), A_w_o.reshape(4, 8 * D, M), B_w1, B_b1, B_w2, B_b2)
    return out.reshape(B, 1, M)
```

```python
import jax
import jax.numpy as jnp
from jax import lax
import jax.experimental.pallas as pl
import jax.experimental.pallas.tpu as pltpu

F32 = jnp.float32
BF16 = jnp.bfloat16

B, H, SK, D, M, DC, F = 2, 32, 16384, 128, 512, 512, 1792
LOG2E = 1.4426950408889634
NT = (((1,), (1,)), ((), ()))

NS = 32
CK = 2048
NC = B * SK // CK

RING = 3
NP = 13
LEAD = 32
WO_SLOTS = ((3, 7), (7, 8))
LAST0 = 3 * D
WO_LAST = (80, 256, 384, 432, 480, 528, 560, 592, 608, 624, 640)

I_WQ, I_WUK, I_C = 0, 2, 4
I_WUV = I_C + NC
I_W1, I_W2, I_SLOTS = I_WUV + 1, I_WUV + 2, I_WUV + 3
I_LAST = I_SLOTS + len(WO_SLOTS)
I_LEAD = I_LAST + len(WO_LAST) - 1
I_X = I_LEAD + 1


def _kernel(x_hbm, ckv_hbm, wq_hbm, wuk_hbm, wuv_hbm, wo_hbm, w1_hbm, b1_hbm, w2_hbm, b2_hbm,
            o_hbm,
            x_buf, b1_buf, b2_buf, c_buf, wq_buf, wuk_buf, wuv_buf, wo_buf, w1_buf, w2_buf, o_buf,
            xf_ref, gate_ref, bc_ref, ring, t8, qa_ref, acc_ref, m_ref, l_ref, a_buf, ctx_ref, sems, sem_in, sem_out):
    def wait_filled(view, i):
        pltpu.make_async_copy(view, view, sems.at[i]).wait()

    def loop(lo, hi, f):
        lax.fori_loop(lo, hi, lambda i, _: f(i), None)

    def start_heads(hbm, buf, i, sem):
        pltpu.make_async_copy(hbm.at[:, pl.ds(i * 4, 4)], buf.at[:, pl.ds(i * 4, 4)], sems.at[sem]).start()

    def start_ckv(t):
        o = pl.multiple_of(t % NS * 32, 32)
        pltpu.make_async_copy(ckv_hbm.at[t // NS, :, pl.ds(o, 32)], c_buf.at[t // 4, pl.ds((t % 4) * 16, 16)],
                              sems.at[I_C + t // 4]).start()

    def wo_rows(blk, o, n):
        return wo_hbm.at[blk, pl.ds(o, n)], wo_buf.at[blk, pl.ds(o, n)]

    def relay(p, out):
        if isinstance(p, int) and p == 0:
            (src, dst), mid = wo_rows(0, LEAD, D - LEAD), ring.at[0, pl.ds(LEAD, D - LEAD)]
        elif isinstance(p, int) and p == NP - 1:
            (src, dst), mid = wo_rows(3, LAST0, WO_LAST[0]), ring.at[p % RING, pl.ds(0, WO_LAST[0])]
        else:
            o = p // 4 * D if isinstance(p, int) else pl.multiple_of(p // 4 * D, D)
            (src, dst), mid = wo_rows(p % 4, o, D), ring.at[p % RING]
        if out:
            return pltpu.make_async_copy(mid, dst, sem_out.at[p % RING])
        return pltpu.make_async_copy(src, mid, sem_in.at[p % RING])

    def relay_step(p):
        dynamic = not isinstance(p, int)
        relay(p, False).wait()
        relay(p, True).start()
        if dynamic or p + 2 < NP:
            if dynamic or p + 2 >= RING:
                relay(p + 2 - RING, True).wait()
            relay(p + 2, False).start(priority=1)

    def broadcast_rows(v, o):
        for b in range(B):
            bc_ref[b, pl.ds(o, 128), :] = jnp.broadcast_to(v[b:b + 1], (128, 128)).T

    small = [pltpu.make_async_copy(a, b, sems.at[I_X]) for a, b in ((x_hbm, x_buf), (b1_hbm, b1_buf), (b2_hbm, b2_buf))]
    lead_src, lead_dst = wo_rows(0, 0, LEAD)
    lead_in = pltpu.make_async_copy(lead_src, ring.at[0, pl.ds(0, LEAD)], sems.at[I_LEAD])
    lead_out = pltpu.make_async_copy(ring.at[0, pl.ds(0, LEAD)], lead_dst, sems.at[I_LEAD])
    for n in range(4):
        pltpu.make_async_copy(wq_hbm.at[n, pl.ds(0, 32)], wq_buf.at[n, pl.ds(0, 32)], sems.at[I_WQ]).start()
        if n == 0:
            lead_in.start(priority=1)
        if n < 2:
            relay(n, False).start(priority=1)
        if n == 0:
            for cp in small:
                cp.start()
    loop(8, 24, lambda i: start_heads(wq_hbm, wq_buf, i, I_WQ + i // 16))

    for cp in small:
        cp.wait()
    x = x_buf[...].astype(F32)
    xc = x - jnp.mean(x, axis=-1, keepdims=True)
    var = jnp.mean(xc * xc, axis=-1, keepdims=True)
    xn = (xc * lax.rsqrt(var + 1e-5)).astype(BF16)
    for j in range(M // 128):
        broadcast_rows(xn.astype(F32)[:, j * 128:(j + 1) * 128], j * 128)
        xf_ref[j] = x_buf[:, j * 128:(j + 1) * 128].astype(F32)
    lead_in.wait()
    lead_out.start()

    q01 = (jnp.zeros((H, D), F32), jnp.zeros((H, D), F32))
    for j in range(2):
        wait_filled(wq_buf.at[:, pl.ds(64 * j, 64)], I_WQ + j)
        if j == 0:
            relay_step(0)
            loop(24, NS, lambda i: start_heads(wq_hbm, wq_buf, i, I_WQ + 1))
            loop(0, 8, lambda i: start_heads(wuk_hbm, wuk_buf, i, I_WUK))
        else:
            lead_out.wait()
            loop(8, 24, lambda i: start_heads(wuk_hbm, wuk_buf, i, I_WUK + i // 16))

        def q_body(i, carry, j=j):
            q0, q1 = carry
            n, r = i // 8, 64 * j + i % 8 * 8
            for u in range(8):
                w = wq_buf[n, r + u].astype(F32)
                q0 = q0 + bc_ref[0, pl.ds(n * 128 + r + u, 1), :] * w
                q1 = q1 + bc_ref[1, pl.ds(n * 128 + r + u, 1), :] * w
            return q0, q1

        q01 = lax.fori_loop(0, 32, q_body, q01)
    q = jnp.concatenate([q01[0], q01[1], jnp.zeros((128 - B * H, D), F32)], axis=0).astype(BF16)

    group = (lax.broadcasted_iota(jnp.int32, (16, 8, 128), 2) % H) // 8
    for j in range(2):
        wait_filled(wuk_buf.at[:, pl.ds(64 * j, 64)], I_WUK + j)
        if j == 0:
            relay_step(1)
            loop(24, NS, lambda i: start_heads(wuk_hbm, wuk_buf, i, I_WUK + 1))
            loop(0, 12, start_ckv)

        def qa_body(i, j=j):
            for s in range(2):
                r0 = 64 * j + (i % 2) * 32 + s * 16
                u = wuk_buf[i // 2, pl.ds(r0, 16)].reshape(16 * H, D)
                r = lax.dot_general(u, q, NT, preferred_element_type=F32).reshape(16, 4, 8, 128)
                v = jnp.where(group == 0, r[:, 0],
                              jnp.where(group == 1, r[:, 1], jnp.where(group == 2, r[:, 2], r[:, 3])))
                t8[pl.ds(pl.multiple_of((i // 2 * 128 + r0) * 8, 128), 128), :] = v.reshape(128, 128)

        loop(0, 8, qa_body)
    sub = lax.broadcasted_iota(jnp.int32, (128, 128), 1) % 8
    for j in range(DC // 128):
        t = t8[pl.ds(j * 1024, 128, stride=8), :]
        for s in range(1, 8):
            t = jnp.where(sub == s, t8[pl.ds(j * 1024 + s, 128, stride=8), :], t)
        qa_ref[:, j * 128:(j + 1) * 128] = (t.T[:B * H] * (D ** -0.5 * LOG2E)).astype(BF16)

    m_ref[...] = jnp.full((B * H, 128), -jnp.inf, F32)
    l_ref[...] = jnp.zeros((B * H, 128), F32)
    acc_ref[...] = jnp.zeros((B * H, DC), F32)

    def chunk(ci):
        wait_filled(c_buf.at[ci], I_C + ci)
        pl.when(ci % 2 == 0)(lambda: relay_step(2 + ci // 2))

        @pl.when(ci + 3 < NC)
        def _():
            for e in range(4):
                start_ckv((ci + 3) * 4 + e)

        @pl.when(ci >= NC - 2)
        def _():
            loop((ci - NC + 2) * 12, (ci - NC + 3) * 12, lambda i: start_heads(wuv_hbm, wuv_buf, i, I_WUV))

        hrows = pl.ds(pl.multiple_of(ci // (NC // B) * H, H), H)
        c = c_buf[ci].reshape(CK, DC)
        sc = lax.dot_general(qa_ref[hrows, :], c, NT, preferred_element_type=F32)
        m_prev = m_ref[hrows, :]
        m_new = jnp.maximum(m_prev, jnp.max(sc, axis=1, keepdims=True))
        p = jnp.exp2(sc - m_new[:, :1])
        alpha = jnp.exp2(m_prev - m_new)
        l_ref[hrows, :] = alpha * l_ref[hrows, :] + jnp.sum(p, axis=1, keepdims=True)
        m_ref[hrows, :] = m_new
        pv = jnp.dot(p.astype(BF16), c, preferred_element_type=F32)
        acc_ref[hrows, :] = acc_ref[hrows, :] * alpha[:, :1] + pv

    loop(0, NC, chunk)

    loop(24, NS, lambda i: start_heads(wuv_hbm, wuv_buf, i, I_WUV))
    w1_copy = pltpu.make_async_copy(w1_hbm, w1_buf, sems.at[I_W1])
    w2_copy = pltpu.make_async_copy(w2_hbm, w2_buf, sems.at[I_W2])
    w1_copy.start()
    w2_copy.start()
    pc = acc_ref[...] / l_ref[...][:, :1]
    lane = lax.broadcasted_iota(jnp.int32, (B * H, 128), 1)
    head = lax.broadcasted_iota(jnp.int32, (B * H, 128), 0) % H
    diag = (lane % H) == head
    for j in range(DC // 128):
        pcj = pc[:, j * 128:(j + 1) * 128]
        for t in range(32):
            rep = jnp.take_along_axis(pcj, lane // H + 4 * t, axis=1)
            a_buf[j, :, t * 128:(t + 1) * 128] = jnp.where(diag, rep, 0.0).astype(BF16)
    relay_step(10)
    wait_filled(wuv_buf, I_WUV)

    for j, (g0, g1) in enumerate(WO_SLOTS):
        def start_slot(k, j=j):
            pltpu.make_async_copy(*wo_rows(pl.ds(0, 3), pl.multiple_of(k * 32, 32), 32), sems.at[I_SLOTS + j]).start()

        loop(4 * g0, 4 * g1, start_slot)
    last = [(pltpu.make_async_copy(*wo_rows(3, LAST0 + lo, hi - lo), sems.at[I_LAST + j]), lo, hi)
            for j, (lo, hi) in enumerate(zip(WO_LAST[:-1], WO_LAST[1:]))]

    def ctx_body(j, ctx):
        return ctx + jnp.dot(a_buf[j], wuv_buf[j].reshape(128 * H, D), preferred_element_type=F32)

    ctx = lax.fori_loop(0, DC // 128, ctx_body, jnp.zeros((B * H, D), F32))
    ctx_ref[...] = jnp.zeros_like(ctx_ref)
    for b in range(B):
        ctx_ref[pl.ds(b, H, stride=8), :] = ctx[b * H:(b + 1) * H]

    w1_copy.wait()
    relay_step(11)
    h = jnp.dot(xn, w1_buf[...], preferred_element_type=F32) + b1_buf[...].astype(F32).reshape(1, F)
    h = jax.nn.gelu(h, approximate=True).astype(BF16)
    w2_copy.wait()
    relay_step(12)
    for cp, _, _ in last:
        cp.start()
    gg = jnp.dot(h, w2_buf[...], preferred_element_type=F32) + b2_buf[...].astype(F32).reshape(1, M)
    gate_ref[...] = gg * jax.nn.sigmoid(gg)

    def ctx_heads(h0, h1):
        return jnp.concatenate([ctx_ref[pl.ds(8 * k, 8), :] for k in range(h0, h1)], axis=1).astype(BF16)

    def project(s, blocks, g0, g1):
        for t in blocks:
            s = s + jnp.dot(ctx_heads(8 * t + g0, 8 * t + g1), wo_buf[t, pl.ds(g0 * D, (g1 - g0) * D), :],
                            preferred_element_type=F32)
        return s

    for g in range(3, 8):
        broadcast_rows(ctx_heads(24 + g, 25 + g).astype(F32), g * D - LAST0)
    s = project(jnp.zeros((8, M), F32), range(4), 0, 2)
    for j, (g0, g1) in enumerate(WO_SLOTS):
        if j == 1:
            for p in range(NP - RING, NP - 1):
                relay(p, True).wait()
            s = project(s, range(4), 2, 3)
        wait_filled(wo_rows(pl.ds(0, 3), g0 * D, (g1 - g0) * D)[1], I_SLOTS + j)
        s = project(s, range(3), g0, g1)
    sub = lax.broadcasted_iota(jnp.int32, (8, 128), 0)
    acc = [[jnp.where(sub == b, s[:, j * 128:(j + 1) * 128], 0.0) for b in range(B)] for j in range(M // 128)]
    for cp, lo, hi in last[:5] + [(relay(NP - 1, True), 0, WO_LAST[0])] + last[5:]:
        cp.wait()
        for r in range(lo, hi, 8):
            cb = [bc_ref[b, pl.ds(r, 8), :] for b in range(B)]
            for j in range(M // 128):
                w = wo_buf[3, pl.ds(LAST0 + r, 8), pl.ds(j * 128, 128)].astype(F32)
                for b in range(B):
                    acc[j][b] = acc[j][b] + w * cb[b]
    even = (sub & 1) == 0
    for j in range(M // 128):
        cols = slice(j * 128, (j + 1) * 128)
        t = jnp.where(even, acc[j][0], acc[j][1]) + pltpu.roll(jnp.where(even, acc[j][1], acc[j][0]), 7, 0)
        t = t + pltpu.roll(t, 2, 0)
        t = t + pltpu.roll(t, 4, 0)
        o_buf[:, cols] = (xf_ref[j] + t[:B] * gate_ref[:, cols]).astype(BF16)
    out = pltpu.make_async_copy(o_buf, o_hbm, sems.at[I_X])
    out.start()
    out.wait()


@jax.jit
def pallas_recurrent_scan__compressed_kv_cla__dense_activation_gelu__decode_kernel(
    A_x: jax.Array,
    A_c_kv: jax.Array,
    A_w_q: jax.Array,
    A_w_uk: jax.Array,
    A_w_uv: jax.Array,
    A_w_o: jax.Array,
    B_x: jax.Array,
    B_w1: jax.Array,
    B_b1: jax.Array,
    B_w2: jax.Array,
    B_b2: jax.Array,
):
    del B_x
    out = pl.pallas_call(
        _kernel,
        out_shape=jax.ShapeDtypeStruct((B, M), BF16),
        in_specs=[pl.BlockSpec(memory_space=pltpu.HBM)] * 10,
        out_specs=pl.BlockSpec(memory_space=pltpu.HBM),
        scratch_shapes=[
            pltpu.VMEM((B, M), BF16), pltpu.VMEM((F,), BF16), pltpu.VMEM((M,), BF16),
            pltpu.VMEM((NC, CK // 32, 32, DC), BF16),
            pltpu.VMEM((4, 128, H, D), BF16), pltpu.VMEM((4, 128, H, D), BF16), pltpu.VMEM((4, 128, H, D), BF16),
            pltpu.VMEM((4, 8 * D, M), BF16), pltpu.VMEM((M, F), BF16), pltpu.VMEM((F, M), BF16),
            pltpu.VMEM((B, M), BF16),
            pltpu.VMEM((M // 128, B, 128), F32), pltpu.VMEM((B, M), F32), pltpu.VMEM((B, WO_LAST[-1], 128), F32),
            pltpu.SMEM((RING, D, M), BF16),
            pltpu.VMEM((DC * 8 + 8, 128), F32),
            pltpu.VMEM((B * H, DC), BF16), pltpu.VMEM((B * H, DC), F32),
            pltpu.VMEM((B * H, 128), F32), pltpu.VMEM((B * H, 128), F32),
            pltpu.VMEM((DC // 128, B * H, 128 * H), BF16),
            pltpu.VMEM((H * 8 + 8, D), F32),
            pltpu.SemaphoreType.DMA((I_X + 1,)), pltpu.SemaphoreType.DMA((RING,)), pltpu.SemaphoreType.DMA((RING,)),
        ],
        compiler_params=pltpu.CompilerParams(vmem_limit_bytes=100 * 1024 * 1024,
                                             disable_bounds_checks=True, disable_semaphore_checks=True),
    )(A_x.reshape(B, M), A_c_kv.reshape(B, 16, 1024, DC), A_w_q.reshape(4, 128, H, D), A_w_uk.reshape(4, 128, H, D),
      A_w_uv.reshape(4, 128, H, D), A_w_o.reshape(4, 8 * D, M), B_w1, B_b1, B_w2, B_b2)
    return out.reshape(B, 1, M)
```
